```python
import jax
import jax.numpy as jnp

def _softmax(x, axis=-1):
    return jax.nn.softmax(x, axis=axis)
def _gelu(x):
    return jax.nn.gelu(x, approximate=True)
def _silu(x):
    return jax.nn.silu(x)
def _sigmoid(x):
    return jax.nn.sigmoid(x)
def _layernorm(x, axis=-1, eps=1e-5):
    m = jnp.mean(x, axis=axis, keepdims=True)
    v = jnp.var(x, axis=axis, keepdims=True)
    return (x - m) / jnp.sqrt(v + eps)
def _scatter_add(tgt, idx, src, axis=0):
    return tgt.at[idx].add(src)
def _segment_sum(src, seg, n):
    return jax.ops.segment_sum(src, seg, n)
class _Rng:
    def __init__(self, key):
        self._k = key
    def _next(self):
        self._k, sub = jax.random.split(self._k)
        return sub
    def normal(self, shape):
        return jax.random.normal(self._next(), shape, dtype=jnp.bfloat16)
    def randint(self, lo, hi, shape):
        return jax.random.randint(self._next(), shape, lo, hi, dtype=jnp.int32)
    def uniform(self, shape, lo=0.0, hi=1.0):
        return jax.random.uniform(self._next(), shape, jnp.bfloat16, lo, hi)
    def permutation(self, n):
        return jax.random.permutation(self._next(), n)


kernel_name = 'gated_mix__sliding_block_cached__moe_arch_mod__decode'

def setup_inputs():
    _rng = _Rng(jax.random.key(int.from_bytes(__import__("os").urandom(4), "little")))
    _w = (lambda a: (lambda t: t.astype(jnp.bfloat16) if jnp.issubdtype(t.dtype, jnp.floating) else t)(jnp.asarray(a)))
    def _A_setup():
        B, Sq, D = 1, 1, 640
        Hq, Hkv, Sk, Dh = 32, 32, 32768, 192
        assert Hq % Hkv == 0, (Hq, Hkv)
        return {
            "x": _w((lambda *s: _rng.normal(s) * 0.05)(B, Sq, D)),
            "k_cache": _w((lambda *s: _rng.normal(s) * 0.05)(B, Hkv, Sk, Dh)),
            "v_cache": _w((lambda *s: _rng.normal(s) * 0.05)(B, Hkv, Sk, Dh)),
            "wq": _w((lambda *s: _rng.normal(s) * 0.05)(D, Hq * Dh) * (D ** -0.5)),
            "wo": _w((lambda *s: _rng.normal(s) * 0.05)(Hq * Dh, D) * ((Hq * Dh) ** -0.5)),
        }
    _A_in = _A_setup()

    def _B_setup():
        B, S, D, F, C = 1, 1, 640, 1536, 1
        return {
            "x": _w((lambda *s: _rng.normal(s) * 0.05)(B, S, D)),
            "w_r": _w((lambda *s: _rng.normal(s) * 0.05)(D)),
            "w_gate": _w((lambda *s: _rng.normal(s) * 0.05)(D, F)),
            "w_up": _w((lambda *s: _rng.normal(s) * 0.05)(D, F)),
            "w_down": _w((lambda *s: _rng.normal(s) * 0.05)(F, D)),
        }
    _B_in = _B_setup()

    return {
        "A_x": _A_in["x"],
        "A_k_cache": _A_in["k_cache"],
        "A_v_cache": _A_in["v_cache"],
        "A_wq": _A_in["wq"],
        "A_wo": _A_in["wo"],
        "B_x": _B_in["x"],
        "B_w_r": _B_in["w_r"],
        "B_w_gate": _B_in["w_gate"],
        "B_w_up": _B_in["w_up"],
        "B_w_down": _B_in["w_down"],
        "gate_w": _w((lambda *s: _rng.normal(s) * 0.05)(640)),
    }

def reference(A_x, A_k_cache, A_v_cache, A_wq, A_wo, B_x, B_w_r, B_w_gate, B_w_up, B_w_down, gate_w):
    def _A_ref(x, k_cache, v_cache, wq, wo):
        B, Sq, D = x.shape
        Hq, Dh = 32, 192
        Hkv, Sk = k_cache.shape[1], k_cache.shape[2]
        W = min(4096, max(256, Sk // 4))
        rep = Hq // Hkv
        q = (lambda x, *d: x.transpose(*d))((x @ wq).reshape(B, Sq, Hq, Dh), 0, 2, 1, 3)
        k = jnp.repeat(k_cache[:, :, Sk - W:, :], rep, axis=1)
        v = jnp.repeat(v_cache[:, :, Sk - W:, :], rep, axis=1)
        scores = jnp.einsum("bhqd,bhkd->bhqk", q, k) * (Dh ** -0.5)
        p = _softmax(scores, axis=-1)
        o = jnp.einsum("bhqk,bhkd->bhqd", p, v)
        return (lambda x, *d: x.transpose(*d))(o, 0, 2, 1, 3).reshape(B, Sq, Hq * Dh) @ wo

    def _B_ref(x, w_r, w_gate, w_up, w_down):
        B, S, D = x.shape
        C = 1
        r = x @ w_r
        idx = jnp.argsort(-r, axis=-1)[:, :C]
        idx_e = jnp.repeat(idx.reshape(B, C, 1), D, axis=2)
        x_sel = jnp.take_along_axis(x, idx_e, axis=1)
        g = _silu(x_sel @ w_gate)
        u = x_sel @ w_up
        y = (g * u) @ w_down
        r_sel = _sigmoid(jnp.take_along_axis(r, idx, axis=1))
        y = y * r_sel.reshape(B, C, 1)
        b_off = (jnp.arange(B) * S).reshape(B, 1)
        flat_idx = (idx + b_off).reshape(B * C)
        zero = (x * 0.0).reshape(B * S, D)
        upd = _scatter_add(zero, flat_idx, y.reshape(B * C, D), axis=0)
        return x + upd.reshape(B, S, D)

    x = A_x
    g = _sigmoid((x * gate_w).sum(-1, keepdims=True))
    a = _A_ref(x, A_k_cache, A_v_cache, A_wq, A_wo)
    b = _B_ref(x, B_w_r, B_w_gate, B_w_up, B_w_down)
    return g * a + (1 - g) * b
```

```python
import jax
import jax.numpy as jnp
import jax.experimental.pallas as pl
import jax.experimental.pallas.tpu as pltpu

H, DH, SK, D, F = 32, 192, 32768, 640, 1536
W = min(4096, max(256, SK // 4))

SEG = 4
LINE = 64
NP = H // 2
RG = 2 * DH // 8
WSEG = W // 128 // SEG
ND, NQ, NF = D // 128, H * DH // 128, F // 128
BIG_LINES = D * H * DH // (1024 * SEG * LINE)
FFN_SEGS = D * F // (1024 * SEG)
FFN_SHARE = FFN_SEGS // NP
FFN_WAYS = dict(wg=NF // SEG, wu=NF // SEG, wd=ND)

KV_RUN, KV_SWEEP = 6, DH // 8
BIG_RUN = 5
SKEW = 26
LAG = 16
END_LAG = 14
WO_GROUP = 8

f32 = jnp.float32
bf16 = jnp.bfloat16


def _sweep(lines, cols, height, run):
    return [(r, c, run) for top in range(0, lines, height) for c in range(cols)
            for r in range(top, top + height, run)]


def _slots(name, hp, units, riders=()):
    out = []
    for i, (r, c, n) in enumerate(units):
        k = i * len(riders) // len(units)
        if (i + 1) * len(riders) // len(units) > k:
            out.append(((name, hp, r, c, n), riders[k]))
        else:
            out.append(((name, hp, r, c, n - 1), (name, hp, r + n - 1, c, 1)))
    return out


def _build_stream():
    kv = _sweep(RG, WSEG, KV_SWEEP, KV_RUN)
    big = _sweep(BIG_LINES, LINE, BIG_LINES, BIG_RUN)
    stream, end = [], {}

    def put(name, hp):
        if hp is None:
            stream.extend(_slots(name, hp, big))
        else:
            ffn = [(w, hp, k, 0, 1) for k in range(FFN_SHARE) for w in FFN_WAYS]
            half = len(ffn) // 2
            stream.extend(_slots(name, hp, kv, ffn[:half] if name == "k" else ffn[half:]))
        end[name, hp] = len(stream)

    put("wq", None)
    put("k", 0)
    for hp in range(1, NP):
        put("k", hp)
        put("v", hp - 1)
    put("v", NP - 1)
    put("wo", None)
    return stream, end, len(kv)


STREAM, END, KV_SLOTS = _build_stream()
N = len(STREAM)
WO_START = END["v", NP - 1]
PACED = N - SKEW - END_LAG

KV_ROWS = RG * WSEG
ROW0 = dict(k=0, v=2 * KV_ROWS, wq=4 * KV_ROWS, wo=4 * KV_ROWS + BIG_LINES * LINE)
ROW0["wg"] = ROW0["wo"] + BIG_LINES * LINE
ROW0["wu"] = ROW0["wg"] + FFN_SEGS
ROW0["wd"] = ROW0["wu"] + FFN_SEGS
BUF_ROWS = ROW0["wd"] + FFN_SEGS
SEM = dict(k=0, v=2, wq=4, ffn=5, small=6, wo=9)


def _kernel(x_hbm, gw_hbm, wr_hbm, k_hbm, v_hbm, wq, wo, wg, wu, wd, out_ref,
            x_v, gw_v, wr_v, buf, q_s, p_s, o_s, h_s, sems, end_sems):
    src = dict(k=k_hbm, v=v_hbm, wq=wq, wo=wo, wg=wg, wu=wu, wd=wd)

    def kv_row(name, hp):
        return ROW0[name] + (hp & 1) * KV_ROWS

    def copy(i, queue, pair):
        name, hp, r, c, n = STREAM[i][1 - queue]
        if name in FFN_WAYS:
            ways = FFN_WAYS[name]
            dst = ROW0[name] + r % ways * (FFN_SEGS // ways) + r // ways + pair(hp) * (FFN_SHARE // ways)
            r, sem = r + pair(hp) * FFN_SHARE, sems.at[SEM["ffn"]]
        elif hp is not None:
            dst, sem = kv_row(name, pair(hp)) + c * RG + r, sems.at[SEM[name] + (pair(hp) & 1)]
            r, c = r + pair(hp) * RG, c + LINE - WSEG
        else:
            dst = ROW0[name] + c * BIG_LINES + r
            if i >= PACED:
                sem = end_sems.at[queue, i - PACED]
            else:
                sem = sems.at[SEM[name] + max(i - WO_START, 0) // WO_GROUP]
        return pltpu.make_async_copy(src[name].at[pl.ds(r, n), pl.ds(c * SEG * 8, SEG * 8)],
                                     buf.at[pl.ds(dst, n)], sem)

    def wait_rows(row0, n, sem):
        rows = buf.at[pl.ds(row0, n)]
        pltpu.make_async_copy(rows, rows, sems.at[sem]).wait()

    small = [pltpu.make_async_copy(a, b, sems.at[SEM["small"] + i])
             for i, (a, b) in enumerate(((x_hbm, x_v), (gw_hbm, gw_v), (wr_hbm, wr_v)))]

    row = jax.lax.broadcasted_iota(jnp.int32, (16, 128), 0)
    lane = jax.lax.broadcasted_iota(jnp.int32, (16, 128), 1)
    st = {}

    def accumulate(key, val):
        st[key] = st[key] + val if key in st else val

    def matmul(lhs, rhs, contract=0):
        return jax.lax.dot_general(lhs.astype(bf16), rhs, (((1,), (contract,)), ((), ())),
                                   preferred_element_type=f32)

    def tiles(row0, n, b):
        return buf[pl.ds(row0, n), b * 8:(b + 1) * 8, :]

    def block(name, kb, c, hp=None):
        if hp is not None:
            blk = tiles(kv_row(name, hp) + c // SEG * RG + kb * 16, 16, c % SEG)
        elif name == "wq":
            at = [divmod(((kb * 16 + a) * NQ + c) // SEG, LINE) for a in range(16)]
            blk = jnp.concatenate([tiles(ROW0[name] + col * BIG_LINES + line, 1, c % SEG) for line, col in at])
        elif name == "wd":
            at = [divmod(ND * v + c, SEG) for v in range(SEG)]
            blk = jnp.stack([tiles(ROW0[name] + way * (FFN_SEGS // ND) + kb * 4, 4, b) for way, b in at], axis=1)
        else:
            blk = tiles(ROW0[name] + c // SEG * (D // 8) + kb * 16, 16, c % SEG)
        return blk.reshape(128, 128)

    def own(g):
        return (row < 8, (row < 8) == (lane < DH - 128), row >= 8)[g]

    def t_token(_):
        for c in small:
            c.wait()
        x = x_v[0].astype(f32)
        st["gate"] = jax.nn.sigmoid(jnp.sum(x * gw_v[...].astype(f32).reshape(1, D), axis=-1, keepdims=True))
        st["route"] = jax.nn.sigmoid(jnp.sum(x * wr_v[...].astype(f32).reshape(1, D), axis=-1, keepdims=True))
        st["x"] = [jnp.broadcast_to(x[:, j * 128:(j + 1) * 128], (16, 128)) for j in range(ND)]

    def t_project(name, c, kb):
        def fn(_):
            accumulate((name, c), matmul(st["x"][kb], block(name, kb, c))[:8])
            if kb == ND - 1 and name == "wq":
                q_s[c] = st.pop((name, c))
            if kb == ND - 1 and name == "wu":
                h_s[c] = jax.nn.silu(st.pop(("wg", c))) * st.pop((name, c))
        return fn

    def t_qk(hp, cg, g, j):
        def fn(pair):
            if j == 0:
                q = q_s[3 * pair(hp) + g]
                st["q"] = jnp.where(own(g), jnp.concatenate([q, q]), 0.0)
            q = st.pop("q") if j == 7 else st["q"]
            accumulate(("s", cg), matmul(jnp.where(row % 8 == j, q, 0.0), block("k", g, 8 * cg + j, pair(hp))))
        return fn

    def t_softmax(_):
        def per_head(vals, op, reduce):
            v = vals[0]
            for u in vals[1:]:
                v = op(v, u)
            v = reduce(v, axis=1, keepdims=True)
            return jnp.where(row < 8, reduce(v[:8], axis=0, keepdims=True), reduce(v[8:], axis=0, keepdims=True))

        s = [st.pop(("s", cg)) * DH ** -0.5 for cg in range(W // 1024)]
        m = per_head(s, jnp.maximum, jnp.max)
        e = [jnp.exp(v - m) for v in s]
        total = per_head(e, jnp.add, jnp.sum)
        for cg, v in enumerate(e):
            p_s[cg] = v / total

    def t_pv(hp, g, cg, j):
        def fn(pair):
            p = jnp.where(row % 8 == j, st["p"][cg], 0.0)
            accumulate("o", matmul(p, block("v", g, 8 * cg + j, pair(hp)), contract=1))
            if (cg, j) == (W // 1024 - 1, 7):
                o = jnp.where(own(g), st.pop("o"), 0.0)
                o = jnp.sum(o[:8] + o[8:], axis=0, keepdims=True) * st["gate"]
                o_s[3 * pair(hp) + g] = jnp.broadcast_to(o, (128, 128)).T
                if g == 2:
                    del st["p"]
        return fn

    def t_down(kb, c):
        def fn(_):
            accumulate("y", matmul(jnp.where(row[:8] == c, h_s[kb], 0.0), block("wd", kb, c)))
            if (kb, c) == (NF - 1, ND - 1):
                y = st.pop("y") * st["route"]
                for j in range(ND):
                    x = st["x"][j][:8]
                    b = x + (x * 0.0 + y)
                    accumulate(("out", j), jnp.where(row[:8] == j, (1.0 - st["gate"]) * b, 0.0))
        return fn

    def t_wo(piece):
        def fn(_):
            _, _, r, c, n = piece
            terms = {}
            for line in range(r, r + n):
                w = buf[ROW0["wo"] + c * BIG_LINES + line].astype(f32)
                o = {}
                for b in range(SEG):
                    rg, j = divmod((line * LINE + c) * SEG + b, ND)
                    if rg not in o:
                        o[rg] = o_s[rg // 16, rg % 16 * 8:(rg % 16 + 1) * 8, :]
                    terms.setdefault(j, []).append(w[b * 8:(b + 1) * 8] * o[rg])
            for j, vals in terms.items():
                while len(vals) > 1:
                    vals = vals[2:] + [vals[0] + vals[1]]
                accumulate(("out", j), vals[0])
        return fn

    n_slots = N + SKEW + END_LAG
    plan = [[] for _ in range(n_slots)]

    def spread(lo, hi, tasks):
        for k, fn in enumerate(tasks):
            plan[lo + k * (hi - lo) // len(tasks)].append(fn)

    def landed(name, hp):
        return END[name, hp] + SKEW + LAG

    def wait_kv(name, hp):
        return lambda pair: wait_rows(kv_row(name, pair(hp)), KV_ROWS, SEM[name] + (pair(hp) & 1))

    def qk_tasks(hp):
        return [wait_kv("k", hp)] + [t_qk(hp, cg, g, j) for cg in range(W // 1024) for g in range(3) for j in range(8)]

    def pv_tasks(hp, *first):
        return ([wait_kv("v", hp), lambda _: st.update(p=[p_s[cg] for cg in range(W // 1024)]), *first]
                + [t_pv(hp, g, cg, j) for g in range(3) for cg in range(W // 1024) for j in range(8)])

    span = KV_SLOTS - 3
    project = [t_project("wq", c, kb) for c in range(NQ) for kb in range(ND)]
    cut = len(project) * 2 // 3
    spread(landed("wq", None), landed("wq", None) + span,
           [lambda _: wait_rows(ROW0["wq"], BIG_LINES * LINE, SEM["wq"]), t_token] + project[:cut])
    spread(landed("k", 0), landed("k", 0) + span, qk_tasks(0) + [t_softmax] + project[cut:])
    for hp in range(1, NP):
        spread(landed("k", hp), landed("k", hp) + span, qk_tasks(hp))
        spread(landed("v", hp - 1), landed("v", hp - 1) + span, pv_tasks(hp - 1, t_softmax))
    assert SKEW + LAG + span <= 2 * KV_SLOTS

    mid = landed("v", NP - 1) + 80
    spread(landed("v", NP - 1), mid,
           pv_tasks(NP - 1, lambda _: wait_rows(ROW0["wg"], 3 * FFN_SEGS, SEM["ffn"]))
           + [t_project(w, c, kb) for c in range(NF) for w in ("wg", "wu") for kb in range(ND)]
           + [t_down(kb, c) for kb in range(NF) for c in range(ND)])
    for i in range(WO_START, N):
        first = i - (i - WO_START) % WO_GROUP
        last = min(first + WO_GROUP, PACED) - 1 if i < PACED else i
        slot = max(last + SKEW + END_LAG, mid + (i - WO_START) // 2)
        if i == first and i < PACED:
            plan[slot].append(lambda _, k=first - WO_START, n=last + 1 - first: wait_rows(
                ROW0["wo"] + k * BIG_RUN, n * BIG_RUN, SEM["wo"] + k // WO_GROUP))
        plan[slot] += [t_wo(STREAM[i][1]), t_wo(STREAM[i][0])]

    def run(lo, hi, pair=lambda hp: hp):
        for i in range(lo, hi):
            done = i - SKEW - END_LAG
            if i < N:
                copy(i, 1, pair).start(priority=1)
            else:
                copy(done, 1, pair).wait()
            if i == 0 or SKEW < i < N + SKEW:
                copy(max(i - SKEW, 0), 0, pair).start(priority=0)
            if i == 2:
                for c in small:
                    c.start()
            if i >= N:
                copy(done, 0, pair).wait()
            for fn in plan[i]:
                fn(pair)

    lo, period = landed("k", 1), 2 * KV_SLOTS
    run(0, lo)

    def body(it, carry):
        run(lo, lo + period, lambda hp: hp + it)
        return carry

    jax.lax.fori_loop(0, NP - 2, body, 0)
    run(lo + period * (NP - 2), n_slots)
    for j in range(ND):
        out_ref[j] = jnp.sum(st["out", j], axis=0, keepdims=True).astype(bf16)


def _tile_order(a, lines):
    r, c = a.shape
    return a.reshape(r // 8, 8, c // 128, 128).transpose(0, 2, 1, 3).reshape(lines, -1, 128)


@jax.jit
def pallas_gated_mix__sliding_block_cached__moe_arch_mod__decode_kernel(
        A_x, A_k_cache, A_v_cache, A_wq, A_wo, B_x, B_w_r, B_w_gate, B_w_up, B_w_down, gate_w):
    del B_x
    caches = [_tile_order(jnp.swapaxes(a, 2, 3).reshape(H * DH, SK), NP * RG) for a in (A_k_cache, A_v_cache)]
    vmem = pltpu.VMEM
    out = pl.pallas_call(
        _kernel,
        out_shape=jax.ShapeDtypeStruct((ND, 1, 128), bf16),
        in_specs=[pl.BlockSpec(memory_space=pl.ANY)] * 10,
        out_specs=pl.BlockSpec(memory_space=pltpu.VMEM),
        scratch_shapes=[
            vmem((1, 1, D), bf16), vmem((D,), bf16), vmem((D,), bf16),
            vmem((BUF_ROWS, SEG * 8, 128), bf16),
            vmem((NQ, 8, 128), f32), vmem((W // 1024, 16, 128), f32),
            vmem((NQ, 128, 128), f32), vmem((NF, 8, 128), f32),
            pltpu.SemaphoreType.DMA((SEM["wo"] + pl.cdiv(PACED - WO_START, WO_GROUP),)),
            pltpu.SemaphoreType.DMA((2, N - PACED)),
        ],
        compiler_params=pltpu.CompilerParams(
            vmem_limit_bytes=64 * 1024 * 1024,
            disable_semaphore_checks=True,
        ),
        name="gated_mix_decode",
    )(A_x, gate_w, B_w_r, *caches, _tile_order(A_wq, BIG_LINES), _tile_order(A_wo, BIG_LINES),
      *[_tile_order(a, FFN_SEGS) for a in (B_w_gate, B_w_up, B_w_down)])
    return out.reshape(1, 1, D)
```

```python
import jax
import jax.numpy as jnp
import jax.experimental.pallas as pl
import jax.experimental.pallas.tpu as pltpu

H, DH, SK, D, F = 32, 192, 32768, 640, 1536
W = min(4096, max(256, SK // 4))

SEG = 4
LINE = 64
NP = H // 2
RG = 2 * DH // 8
WSEG = W // 128 // SEG
ND, NQ, NF = D // 128, H * DH // 128, F // 128
BIG_LINES = D * H * DH // (1024 * SEG * LINE)
FFN_SEGS = D * F // (1024 * SEG)
FFN_SHARE = FFN_SEGS // NP
FFN_WAYS = dict(wg=NF // SEG, wu=NF // SEG, wd=ND)

KV_RUN, KV_SWEEP = 6, DH // 8
BIG_RUN = 5
TAIL, TAIL_RUN = 16, 4
Q0_SEGS = 1
SKEW = 26
LAG = 16
END_LAG = 13
WO_GROUP = 8

f32 = jnp.float32
bf16 = jnp.bfloat16


def _sweep(top, bottom, cols, run):
    return [(r, c, min(run, bottom - r), True) for c in cols for r in range(top, bottom, run)]


def _slots(name, hp, units, riders=()):
    out = []
    for i, (r, c, n, down) in enumerate(units):
        k = i * len(riders) // len(units)
        if (i + 1) * len(riders) // len(units) > k:
            out.append(((name, hp, r, c, n, down), riders[k]))
        else:
            m = n - Q0_SEGS
            out.append(((name, hp, r, c, m, down), (name, hp, r + m * down, c + m * (not down), n - m, down)))
    return out


def _build_stream():
    kv = [u for top in range(0, RG, KV_SWEEP) for u in _sweep(top, top + KV_SWEEP, range(WSEG), KV_RUN)]
    stream, end = [], {}

    def put(name, hp, units):
        ffn = [(w, hp, k, 0, 1, True) for k in range(FFN_SHARE) for w in FFN_WAYS]
        riders = dict(k=ffn[:len(ffn) // 2], v=ffn[len(ffn) // 2:]).get(name, ())
        stream.extend(_slots(name, hp, units, riders))
        end[name, hp] = len(stream)

    put("wq", None, _sweep(0, BIG_LINES, range(LINE), BIG_RUN))
    put("k", 0, kv)
    for hp in range(1, NP):
        put("k", hp, kv)
        put("v", hp - 1, kv)
    put("v", NP - 1, kv)
    put("wo", None, _sweep(0, BIG_LINES, range(LINE - TAIL), BIG_RUN)
        + _sweep(0, BIG_LINES - 1, range(LINE - TAIL, LINE), BIG_RUN)
        + [(BIG_LINES - 1, c, TAIL_RUN, False) for c in range(LINE - TAIL, LINE, TAIL_RUN)])
    return stream, end, len(kv)


STREAM, END, KV_SLOTS = _build_stream()
N = len(STREAM)
WO_START = END["v", NP - 1]
PACED = N - SKEW - END_LAG

KV_ROWS = RG * WSEG
ROW0 = dict(k=0, v=2 * KV_ROWS, wq=4 * KV_ROWS, wo=4 * KV_ROWS + BIG_LINES * LINE)
ROW0["wg"] = ROW0["wo"] + BIG_LINES * LINE
ROW0["wu"] = ROW0["wg"] + FFN_SEGS
ROW0["wd"] = ROW0["wu"] + FFN_SEGS
BUF_ROWS = ROW0["wd"] + FFN_SEGS
WO_ROW = [ROW0["wo"]]
for _slot in STREAM[WO_START:]:
    WO_ROW.append(WO_ROW[-1] + _slot[0][4] + _slot[1][4])
SEM = dict(k=0, v=2, wq=4, ffn=5, small=6, wo=9)


def _kernel(x_hbm, gw_hbm, wr_hbm, k_hbm, v_hbm, wq, wo, wg, wu, wd, out_ref,
            x_v, gw_v, wr_v, buf, q_s, p_s, o_s, h_s, sems, end_sems):
    src = dict(k=k_hbm, v=v_hbm, wq=wq, wo=wo, wg=wg, wu=wu, wd=wd)

    def kv_row(name, hp):
        return ROW0[name] + (hp & 1) * KV_ROWS

    def wo_row(i, queue):
        return WO_ROW[i - WO_START] + (0 if queue else STREAM[i][0][4])

    def copy(i, queue, pair):
        name, hp, r, c, n, down = STREAM[i][1 - queue]
        if name in FFN_WAYS:
            ways = FFN_WAYS[name]
            dst = ROW0[name] + r % ways * (FFN_SEGS // ways) + r // ways + pair(hp) * (FFN_SHARE // ways)
            r, sem = r + pair(hp) * FFN_SHARE, sems.at[SEM["ffn"]]
        elif hp is not None:
            dst, sem = kv_row(name, pair(hp)) + (c * RG + r), sems.at[SEM[name] + (pair(hp) & 1)]
            r, c = r + pair(hp) * RG, c + LINE - WSEG
        elif name == "wq":
            dst, sem = ROW0[name] + c * BIG_LINES + r, sems.at[SEM[name]]
        else:
            dst = wo_row(i, queue)
            sem = end_sems.at[queue, i - PACED] if i >= PACED else sems.at[SEM[name] + (i - WO_START) // WO_GROUP]
        piece = src[name].at[pl.ds(r, n), c] if down else src[name].at[r, pl.ds(c, n)]
        return pltpu.make_async_copy(piece, buf.at[pl.ds(dst, n)], sem)

    def wait_rows(row0, n, sem):
        rows = buf.at[pl.ds(row0, n)]
        pltpu.make_async_copy(rows, rows, sems.at[sem]).wait()

    small = [pltpu.make_async_copy(a, b, sems.at[SEM["small"] + i])
             for i, (a, b) in enumerate(((x_hbm, x_v), (gw_hbm, gw_v), (wr_hbm, wr_v)))]

    row = jax.lax.broadcasted_iota(jnp.int32, (16, 128), 0)
    lane = jax.lax.broadcasted_iota(jnp.int32, (16, 128), 1)
    pick = [(row & 7) == j for j in range(8)]
    st = {}

    def accumulate(key, val):
        st[key] = jax.lax.add(st[key], val) if key in st else val

    def matmul(lhs, rhs, contract=0):
        return jax.lax.dot_general(lhs.astype(bf16), rhs, (((1,), (contract,)), ((), ())),
                                   preferred_element_type=f32)

    def tiles(row0, n, b):
        return buf[pl.ds(row0, n), b * 8:(b + 1) * 8, :]

    def block(name, kb, c, hp=None):
        if hp is not None:
            blk = tiles(kv_row(name, hp) + c // SEG * RG + kb * 16, 16, c % SEG)
        elif name == "wq":
            at = [divmod(((kb * 16 + a) * NQ + c) // SEG, LINE) for a in range(16)]
            blk = jnp.concatenate([tiles(ROW0[name] + col * BIG_LINES + line, 1, c % SEG) for line, col in at])
        elif name == "wd":
            at = [divmod(ND * v + c, SEG) for v in range(SEG)]
            blk = jnp.stack([tiles(ROW0[name] + way * (FFN_SEGS // ND) + kb * 4, 4, b) for way, b in at], axis=1)
        else:
            blk = tiles(ROW0[name] + c // SEG * (D // 8) + kb * 16, 16, c % SEG)
        return blk.reshape(128, 128)

    def own(g):
        return (row < 8, (row < 8) == (lane < DH - 128), row >= 8)[g]

    def t_token(_):
        for c in small:
            c.wait()
        x = x_v[0].astype(f32)
        st["gate"] = jax.nn.sigmoid(jnp.sum(x * gw_v[...].astype(f32).reshape(1, D), axis=-1, keepdims=True))
        st["route"] = jax.nn.sigmoid(jnp.sum(x * wr_v[...].astype(f32).reshape(1, D), axis=-1, keepdims=True))
        st["x"] = [jnp.broadcast_to(x[:, j * 128:(j + 1) * 128], (16, 128)) for j in range(ND)]

    def t_project(name, c, kb):
        def fn(_):
            accumulate((name, c), matmul(st["x"][kb], block(name, kb, c))[:8])
            if kb == ND - 1 and name == "wq":
                q_s[c] = st.pop((name, c))
            if kb == ND - 1 and name == "wu":
                h_s[c] = jax.nn.silu(st.pop(("wg", c))) * st.pop((name, c))
        return fn

    def t_qk(hp, cg, g, j):
        def fn(pair):
            if j == 0:
                q = q_s[3 * pair(hp) + g]
                st["q"] = jnp.where(own(g), jnp.concatenate([q, q]), 0.0)
            q = st.pop("q") if j == 7 else st["q"]
            accumulate(("s", cg), matmul(jnp.where(pick[j], q, 0.0), block("k", g, 8 * cg + j, pair(hp))))
        return fn

    def t_softmax(_):
        def per_head(vals, op, reduce):
            v = vals[0]
            for u in vals[1:]:
                v = op(v, u)
            v = reduce(v, axis=1, keepdims=True)
            return jnp.where(row < 8, reduce(v[:8], axis=0, keepdims=True), reduce(v[8:], axis=0, keepdims=True))

        s = [st.pop(("s", cg)) * DH ** -0.5 for cg in range(W // 1024)]
        m = per_head(s, jnp.maximum, jnp.max)
        e = [jnp.exp(v - m) for v in s]
        total = per_head(e, jnp.add, jnp.sum)
        for cg, v in enumerate(e):
            p_s[cg] = v / total

    def t_pv(hp, g, cg, j):
        def fn(pair):
            p = jnp.where(pick[j], st["p"][cg], 0.0)
            accumulate("o", matmul(p, block("v", g, 8 * cg + j, pair(hp)), contract=1))
            if (cg, j) == (W // 1024 - 1, 7):
                o = jnp.where(own(g), st.pop("o"), 0.0)
                o = jnp.sum(o[:8] + o[8:], axis=0, keepdims=True) * st["gate"]
                o_s[3 * pair(hp) + g] = jnp.broadcast_to(o, (128, 128)).T
                if g == 2:
                    del st["p"]
        return fn

    def t_down(kb, c):
        def fn(_):
            accumulate("y", matmul(jnp.where(row[:8] == c, h_s[kb], 0.0), block("wd", kb, c)))
            if (kb, c) == (NF - 1, ND - 1):
                y = st.pop("y") * st["route"]
                for j in range(ND):
                    x = st["x"][j][:8]
                    b = x + (x * 0.0 + y)
                    accumulate(("out", j), jnp.where(row[:8] == j, (1.0 - st["gate"]) * b, 0.0))
        return fn

    def t_wo(i, queue):
        def fn(_):
            _, _, r, c, n, down = STREAM[i][1 - queue]
            w = buf[pl.ds(wo_row(i, queue), n)].astype(f32).reshape(n * SEG, 8, 128)
            terms, o = {}, {}
            for t in range(n * SEG):
                rg, j = divmod((r * LINE + c + t // SEG * (LINE if down else 1)) * SEG + t % SEG, ND)
                if rg not in o:
                    o[rg] = o_s[rg // 16, rg % 16 * 8:(rg % 16 + 1) * 8, :]
                terms.setdefault(j, []).append(jax.lax.mul(jax.lax.index_in_dim(w, t, keepdims=False), o[rg]))
            for j, vals in terms.items():
                while len(vals) > 1:
                    vals = vals[2:] + [jax.lax.add(vals[0], vals[1])]
                accumulate(("out", j), vals[0])
        return fn

    n_slots = N + SKEW + END_LAG
    plan = [[] for _ in range(n_slots)]

    def spread(lo, hi, tasks):
        for k, fn in enumerate(tasks):
            plan[lo + k * (hi - lo) // len(tasks)].append(fn)

    def landed(name, hp):
        return END[name, hp] + SKEW + LAG

    def wait_kv(name, hp):
        return lambda pair: wait_rows(kv_row(name, pair(hp)), KV_ROWS, SEM[name] + (pair(hp) & 1))

    def qk_tasks(hp):
        return [wait_kv("k", hp)] + [t_qk(hp, cg, g, j) for cg in range(W // 1024) for g in range(3) for j in range(8)]

    def pv_tasks(hp, *first):
        return ([wait_kv("v", hp), lambda _: st.update(p=[p_s[cg] for cg in range(W // 1024)]), *first]
                + [t_pv(hp, g, cg, j) for g in range(3) for cg in range(W // 1024) for j in range(8)])

    span = KV_SLOTS - 3
    project = [t_project("wq", c, kb) for c in range(NQ) for kb in range(ND)]
    cut = len(project) * 2 // 3
    spread(landed("wq", None), landed("wq", None) + span,
           [lambda _: wait_rows(ROW0["wq"], BIG_LINES * LINE, SEM["wq"]), t_token] + project[:cut])
    spread(landed("k", 0), landed("k", 0) + span, qk_tasks(0) + [t_softmax] + project[cut:])
    for hp in range(1, NP):
        spread(landed("k", hp), landed("k", hp) + span, qk_tasks(hp))
        spread(landed("v", hp - 1), landed("v", hp - 1) + span, pv_tasks(hp - 1, t_softmax))
    assert SKEW + LAG + span <= 2 * KV_SLOTS

    mid = landed("v", NP - 1) + 80
    spread(landed("v", NP - 1), mid,
           pv_tasks(NP - 1, lambda _: wait_rows(ROW0["wg"], 3 * FFN_SEGS, SEM["ffn"]))
           + [t_project(w, c, kb) for c in range(NF) for w in ("wg", "wu") for kb in range(ND)]
           + [t_down(kb, c) for kb in range(NF) for c in range(ND)])
    for i in range(WO_START, N):
        first = i - (i - WO_START) % WO_GROUP
        last = min(first + WO_GROUP, PACED) - 1 if i < PACED else i
        slot = max(last + SKEW + END_LAG, mid + (i - WO_START) // 2)
        if i == first and i < PACED:
            plan[slot].append(lambda _, a=first - WO_START, b=last + 1 - WO_START: wait_rows(
                WO_ROW[a], WO_ROW[b] - WO_ROW[a], SEM["wo"] + a // WO_GROUP))
        plan[slot] += [t_wo(i, 0), t_wo(i, 1)]

    def run(lo, hi, pair=lambda hp: hp):
        for i in range(lo, hi):
            done = i - SKEW - END_LAG
            if i < N:
                copy(i, 1, pair).start(priority=1)
            else:
                copy(done, 1, pair).wait()
            if i == 0 or SKEW < i < N + SKEW:
                copy(max(i - SKEW, 0), 0, pair).start(priority=0)
            if i == 2:
                for c in small:
                    c.start()
            if i >= N:
                copy(done, 0, pair).wait()
            for fn in plan[i]:
                fn(pair)

    lo, period = landed("k", 1), 2 * KV_SLOTS
    run(0, lo)

    def body(it, carry):
        run(lo, lo + period, lambda hp: hp + it)
        return carry

    jax.lax.fori_loop(0, NP - 2, body, 0)
    run(lo + period * (NP - 2), n_slots)
    for j in range(ND):
        out_ref[j] = jnp.sum(st["out", j], axis=0, keepdims=True).astype(bf16)


def _tile_order(a, lines):
    r, c = a.shape
    return a.reshape(r // 8, 8, c // 128, 128).transpose(0, 2, 1, 3).reshape(lines, -1, SEG * 8, 128)


@jax.jit
def pallas_gated_mix__sliding_block_cached__moe_arch_mod__decode_kernel(
        A_x, A_k_cache, A_v_cache, A_wq, A_wo, B_x, B_w_r, B_w_gate, B_w_up, B_w_down, gate_w):
    del B_x
    caches = [_tile_order(jnp.swapaxes(a, 2, 3).reshape(H * DH, SK), NP * RG) for a in (A_k_cache, A_v_cache)]
    vmem = pltpu.VMEM
    out = pl.pallas_call(
        _kernel,
        out_shape=jax.ShapeDtypeStruct((ND, 1, 128), bf16),
        in_specs=[pl.BlockSpec(memory_space=pl.ANY)] * 10,
        out_specs=pl.BlockSpec(memory_space=pltpu.VMEM),
        scratch_shapes=[
            vmem((1, 1, D), bf16), vmem((D,), bf16), vmem((D,), bf16),
            vmem((BUF_ROWS, SEG * 8, 128), bf16),
            vmem((NQ, 8, 128), f32), vmem((W // 1024, 16, 128), f32),
            vmem((NQ, 128, 128), f32), vmem((NF, 8, 128), f32),
            pltpu.SemaphoreType.DMA((SEM["wo"] + pl.cdiv(PACED - WO_START, WO_GROUP),)),
            pltpu.SemaphoreType.DMA((2, N - PACED)),
        ],
        compiler_params=pltpu.CompilerParams(
            vmem_limit_bytes=64 * 1024 * 1024,
            disable_semaphore_checks=True,
        ),
        name="gated_mix_decode",
    )(A_x, gate_w, B_w_r, *caches, _tile_order(A_wq, BIG_LINES), _tile_order(A_wo, BIG_LINES),
      *[_tile_order(a, FFN_SEGS) for a in (B_w_gate, B_w_up, B_w_down)])
    return out.reshape(1, 1, D)
```

```python
import jax
import jax.numpy as jnp
import jax.experimental.pallas as pl
import jax.experimental.pallas.tpu as pltpu

H, DH, SK, D, F = 32, 192, 32768, 640, 1536
W = min(4096, max(256, SK // 4))

SEG = 4
LINE = 64
NP = H // 2
RG = 2 * DH // 8
WSEG = W // 128 // SEG
ND, NQ, NF = D // 128, H * DH // 128, F // 128
BIG_LINES = D * H * DH // (1024 * SEG * LINE)
FFN_SEGS = D * F // (1024 * SEG)
FFN_SHARE = FFN_SEGS // NP
FFN_WAYS = dict(wg=NF // SEG, wu=NF // SEG, wd=ND)

KV_RUN, KV_SWEEP = 6, 12
KV_COLS = ((7, 4), (6, 5), (3, 0), (2, 1))
BIG_RUN = 5
TAIL, TAIL_RUN = 16, 4
SKEW = 26
LAG = 16
END_LAG = 13

f32 = jnp.float32
bf16 = jnp.bfloat16


def _sweep(top, bottom, cols, run):
    return [(r, c, min(run, bottom - r), True) for c in cols for r in range(top, bottom, run)]


def _slots(name, hp, units, riders=()):
    out = []
    for i, (r, c, n, down) in enumerate(units):
        k = i * len(riders) // len(units)
        if (i + 1) * len(riders) // len(units) > k:
            out.append(((name, hp, r, c, n, down), riders[k]))
        else:
            m = n - 1
            out.append(((name, hp, r, c, m, down), (name, hp, r + m * down, c + m * (not down), n - m, down)))
    return out


def _build_stream():
    kv = [u for cols in KV_COLS for top in range(0, RG, KV_SWEEP)
          for u in _sweep(top, top + KV_SWEEP, cols, KV_RUN)]
    stream, end = [], {}

    def put(name, hp, units):
        ffn = [(w, hp, k, 0, 1, True) for k in range(FFN_SHARE) for w in FFN_WAYS]
        riders = dict(k=ffn[:len(ffn) // 2], v=ffn[len(ffn) // 2:]).get(name, ())
        stream.extend(_slots(name, hp, units, riders))
        end[name, hp] = len(stream)

    put("wq", None, _sweep(0, BIG_LINES, range(LINE), BIG_RUN))
    put("k", 0, kv)
    for hp in range(1, NP):
        put("k", hp, kv)
        put("v", hp - 1, kv)
    put("v", NP - 1, kv)
    put("wo", None, _sweep(0, BIG_LINES, range(LINE - TAIL), BIG_RUN)
        + _sweep(0, BIG_LINES - 1, range(LINE - TAIL, LINE), BIG_RUN)
        + [(BIG_LINES - 1, c, TAIL_RUN, False) for c in range(LINE - TAIL, LINE, TAIL_RUN)])
    return stream, end, len(kv)


STREAM, END, KV_SLOTS = _build_stream()
N = len(STREAM)
WO_START = END["v", NP - 1]
COL_SLOTS = BIG_LINES // BIG_RUN
WO_GROUPS = (LINE - TAIL) // ND
FINE = WO_START + WO_GROUPS * ND * COL_SLOTS

KV_ROWS = RG * WSEG
ROW0 = dict(k=0, v=2 * KV_ROWS, wq=4 * KV_ROWS, wo=4 * KV_ROWS + BIG_LINES * LINE)
ROW0["wg"] = ROW0["wo"] + BIG_LINES * LINE
ROW0["wu"] = ROW0["wg"] + FFN_SEGS
ROW0["wd"] = ROW0["wu"] + FFN_SEGS
BUF_ROWS = ROW0["wd"] + FFN_SEGS
WO_ROW = [ROW0["wo"]]
for _slot in STREAM[WO_START:]:
    WO_ROW.append(WO_ROW[-1] + _slot[0][4] + _slot[1][4])
SEM = dict(k=0, v=2, wq=4, ffn=5, small=6, wo=9)


def _kernel(x_hbm, gw_hbm, wr_hbm, k_hbm, v_hbm, wq, wo, wg, wu, wd, out_ref,
            x_v, gw_v, wr_v, buf, q_s, p_s, o_s, h_s, sems, end_sems):
    src = dict(k=k_hbm, v=v_hbm, wq=wq, wo=wo, wg=wg, wu=wu, wd=wd)

    def kv_row(name, hp):
        return ROW0[name] + (hp & 1) * KV_ROWS

    def wo_row(i, queue):
        return WO_ROW[i - WO_START] + (0 if queue else STREAM[i][0][4])

    def copy(i, queue, step):
        name, hp, r, c, n, down = STREAM[i][1 - queue]
        if name in FFN_WAYS:
            ways = FFN_WAYS[name]
            dst = ROW0[name] + r % ways * (FFN_SEGS // ways) + r // ways + (hp + step) * (FFN_SHARE // ways)
            r, sem = r + (hp + step) * FFN_SHARE, sems.at[SEM["ffn"]]
        elif name == "wq":
            c = c + step
            dst, sem = ROW0[name] + r + c * BIG_LINES, sems.at[SEM[name]]
        elif name == "wo":
            dst = wo_row(i, queue)
            group = (i - WO_START) // (ND * COL_SLOTS)
            sem = end_sems.at[queue, i - FINE] if i >= FINE else sems.at[SEM[name] + group]
        else:
            hp = hp + step
            dst, sem = kv_row(name, hp) + (c * RG + r), sems.at[SEM[name] + (hp & 1)]
            r, c = r + hp * RG, c + LINE - WSEG
        piece = src[name].at[pl.ds(r, n), c] if down else src[name].at[r, pl.ds(c, n)]
        return pltpu.make_async_copy(piece, buf.at[pl.ds(dst, n)], sem)

    def wait_rows(row0, n, sem):
        rows = buf.at[pl.ds(row0, n)]
        pltpu.make_async_copy(rows, rows, sems.at[sem]).wait()

    small = [pltpu.make_async_copy(a, b, sems.at[SEM["small"] + i])
             for i, (a, b) in enumerate(((x_hbm, x_v), (gw_hbm, gw_v), (wr_hbm, wr_v)))]

    row = jax.lax.broadcasted_iota(jnp.int32, (16, 128), 0)
    lane = jax.lax.broadcasted_iota(jnp.int32, (16, 128), 1)
    st = {}

    def accumulate(key, val):
        st[key] = jax.lax.add(st[key], val) if key in st else val

    def matmul(lhs, rhs, contract=0):
        return jax.lax.dot_general(lhs.astype(bf16), rhs, (((1,), (contract,)), ((), ())),
                                   preferred_element_type=f32)

    def kv_matmul(name, hp, g, col, lhs, contract):
        blk = buf[pl.ds(kv_row(name, hp) + (col * RG + g * 16), 16)]
        out = [matmul(jnp.where((row & 7) == (col * SEG + b) % 8, lhs, 0.0), blk[:, b].reshape(128, 128), contract)
               for b in range(SEG)]
        return (out[0] + out[1]) + (out[2] + out[3])

    def every(stride, first, *index):
        rows = buf[(pl.ds(first, (ND - 1) * stride + 1), *index)]
        return jnp.concatenate([jax.lax.index_in_dim(rows, u * stride) for u in range(ND)])

    def own(g):
        return (row < 8, (row < 8) == (lane < DH - 128), row >= 8)[g]

    def t_token(_):
        for c in small:
            c.wait()
        x = x_v[0].astype(f32)
        st["gate"] = jax.nn.sigmoid(jnp.sum(x * gw_v[...].astype(f32).reshape(1, D), axis=-1, keepdims=True))
        st["route"] = jax.nn.sigmoid(jnp.sum(x * wr_v[...].astype(f32).reshape(1, D), axis=-1, keepdims=True))
        st["x"] = jnp.broadcast_to(x, (8, D))

    def t_q(hp, g):
        def fn(step):
            c = 3 * (hp + step) + g
            seg, b = c >> 2, c & (SEG - 1)
            parts = []
            for v in range(16):
                at = seg + v * NQ // SEG
                first = ROW0["wq"] + (at & (LINE - 1)) * BIG_LINES + (at >> 6)
                parts.append(every(BIG_LINES // ND, first, b))
            q_s[g] = matmul(st["x"], jnp.stack(parts, axis=1).reshape(D, 128))
        return fn

    def t_qk(hp, col, g):
        def fn(step):
            q = q_s[g]
            q = jnp.where(own(g), jnp.concatenate([q, q]), 0.0)
            accumulate(("s", col * SEG // 8), kv_matmul("k", hp + step, g, col, q, 0))
        return fn

    def t_softmax(_):
        def per_head(vals, op, reduce):
            v = vals[0]
            for u in vals[1:]:
                v = op(v, u)
            v = reduce(v, axis=1, keepdims=True)
            return jnp.where(row < 8, reduce(v[:8], axis=0, keepdims=True), reduce(v[8:], axis=0, keepdims=True))

        s = [st.pop(("s", cg)) * DH ** -0.5 for cg in range(W // 1024)]
        m = per_head(s, jnp.maximum, jnp.max)
        e = [jnp.exp(v - m) for v in s]
        total = per_head(e, jnp.add, jnp.sum)
        for cg, v in enumerate(e):
            p_s[cg] = v / total

    def t_pv(hp, g, col):
        def fn(step):
            accumulate("o", kv_matmul("v", hp + step, g, col, st["p"][col * SEG // 8], 1))
            if col == WSEG - 1:
                o = jnp.where(own(g), st.pop("o"), 0.0)
                o = jnp.sum(o[:8] + o[8:], axis=0, keepdims=True) * st["gate"]
                o = jnp.broadcast_to(o, (128, 128)).T
                o_s[pl.ds((hp + step) * RG + g * 16, 16)] = o.reshape(16, 8, 128)
                if g == 2:
                    del st["p"]
        return fn

    def t_up(name, c):
        def fn(_):
            w = buf[pl.ds(ROW0[name] + c // SEG * (D // 8), D // 8), c % SEG]
            st[name] = matmul(st["x"], w.reshape(D, 128))
            if name == "wu":
                h_s[:, c * 128:(c + 1) * 128] = jax.nn.silu(st.pop("wg")) * st.pop("wu")
        return fn

    def t_down(j, k):
        def fn(_):
            at = [divmod(ND * v + j, SEG) for v in range(SEG)]
            w = [buf[pl.ds(ROW0["wd"] + way * (FFN_SEGS // ND) + k * 16, 16), b] for way, b in at]
            accumulate("y", matmul(h_s[:, k * 512:(k + 1) * 512], jnp.stack(w, axis=1).reshape(512, 128)))
            if k == F // 512 - 1:
                x = st["x"][:, j * 128:(j + 1) * 128]
                b = x + (x * 0.0 + st.pop("y") * st["route"])
                accumulate(("out", j), jnp.where(row[:8] == 0, (1.0 - st["gate"]) * b, 0.0))
        return fn

    def apply_wo(w, line, col):
        n = w.shape[0] * SEG
        rg, j0 = divmod((line * LINE + col) * SEG, ND)
        groups = pl.cdiv(j0 + n, ND)
        o = jnp.broadcast_to(o_s[pl.ds(rg, groups)][:, None], (groups, ND, 8, 128))
        terms = w.astype(f32).reshape(n, 8, 128) * o.reshape(groups * ND, 8, 128)[j0:j0 + n]
        if n % ND == 0:
            terms = jnp.sum(terms.reshape(n // ND, ND, 8, 128), axis=0)
        for t in range(terms.shape[0]):
            accumulate(("out", (j0 + t) % ND), jax.lax.index_in_dim(terms, t, keepdims=False))

    def t_wo_line(group, line):
        first = ROW0["wo"] + group * ND * BIG_LINES + line
        return lambda _: apply_wo(every(BIG_LINES, first), line, group * ND)

    def wo_piece(i, queue):
        _, _, r, c, n, down = STREAM[i][1 - queue]
        w = buf[pl.ds(wo_row(i, queue), n)]
        if down:
            for k in range(n):
                apply_wo(w[k:k + 1], r + k, c)
        else:
            apply_wo(w, r, c)

    n_slots = N + SKEW + END_LAG
    plan = [[] for _ in range(n_slots)]

    def spread(lo, hi, tasks):
        for k, fn in enumerate(tasks):
            plan[lo + k * (hi - lo) // len(tasks)].append(fn)

    def landed(name, hp):
        return END[name, hp] + SKEW + LAG

    def wait_kv(name, hp):
        return lambda step: wait_rows(kv_row(name, hp + step), KV_ROWS, SEM[name] + ((hp + step) & 1))

    def q_tasks(hp):
        return [t_q(hp, g) for g in range(3)] if hp < NP else []

    def qk_tasks(hp):
        return [wait_kv("k", hp)] + [t_qk(hp, col, g) for col in range(WSEG) for g in range(3)]

    def pv_tasks(hp, first):
        return ([wait_kv("v", hp), lambda _: st.update(p=[p_s[cg] for cg in range(W // 1024)]), first]
                + [t_pv(hp, g, col) for g in range(3) for col in range(WSEG)])

    span = KV_SLOTS - 1
    spread(landed("wq", None), landed("wq", None) + span,
           [lambda _: wait_rows(ROW0["wq"], BIG_LINES * LINE, SEM["wq"]), t_token] + q_tasks(0))
    spread(landed("k", 0), landed("k", 0) + span, qk_tasks(0) + [t_softmax] + q_tasks(1))
    for hp in range(1, NP):
        spread(landed("k", hp), landed("k", hp) + span, qk_tasks(hp))
        spread(landed("v", hp - 1), landed("v", hp - 1) + span, pv_tasks(hp - 1, t_softmax) + q_tasks(hp + 1))
    assert SKEW + LAG + span <= 2 * KV_SLOTS

    mid = landed("v", NP - 1) + 80
    spread(landed("v", NP - 1), mid,
           pv_tasks(NP - 1, lambda _: wait_rows(ROW0["wg"], 3 * FFN_SEGS, SEM["ffn"]))
           + [t_up(w, c) for c in range(NF) for w in ("wg", "wu")]
           + [t_down(j, k) for j in range(ND) for k in range(F // 512)])
    for group in range(WO_GROUPS):
        lo = max(WO_START + (group + 1) * ND * COL_SLOTS + SKEW + LAG, mid + 8 * group)
        plan[lo].append(lambda _, group=group: wait_rows(
            ROW0["wo"] + group * ND * BIG_LINES, ND * BIG_LINES, SEM["wo"] + group))
        spread(lo, lo + 8, [t_wo_line(group, line) for line in range(BIG_LINES)])
    assert mid <= FINE + SKEW + END_LAG <= N

    def run(lo, hi, step=0):
        for i in range(lo, hi):
            done = i - SKEW - END_LAG
            if i < N:
                copy(i, 1, step).start(priority=1)
            if done >= FINE:
                copy(done, 1, step).wait()
            if i == 0 or SKEW < i < N + SKEW:
                copy(max(i - SKEW, 0), 0, step).start(priority=0)
            if i == 2:
                for c in small:
                    c.start()
            if done >= FINE:
                copy(done, 0, step).wait()
                wo_piece(done, 0)
                wo_piece(done, 1)
            for fn in plan[i]:
                fn(step)

    def loop(lo, period, count):
        def body(step, carry):
            run(lo, lo + period, step)
            return carry
        jax.lax.fori_loop(0, count, body, 0)
        return lo + period * count

    run(0, SKEW + 1)
    at = loop(SKEW + 1, COL_SLOTS, (END["wq", None] - SKEW - 1) // COL_SLOTS)
    run(at, landed("k", 1))
    at = loop(landed("k", 1), 2 * KV_SLOTS, NP - 2)
    run(at, n_slots)
    for j in range(ND):
        out_ref[j] = jnp.sum(st["out", j], axis=0, keepdims=True).astype(bf16)


def _tile_order(a, lines):
    r, c = a.shape
    return a.reshape(r // 8, 8, c // 128, 128).transpose(0, 2, 1, 3).reshape(lines, -1, SEG, 8, 128)


@jax.jit
def pallas_gated_mix__sliding_block_cached__moe_arch_mod__decode_kernel(
        A_x, A_k_cache, A_v_cache, A_wq, A_wo, B_x, B_w_r, B_w_gate, B_w_up, B_w_down, gate_w):
    del B_x
    caches = [_tile_order(jnp.swapaxes(a, 2, 3).reshape(H * DH, SK), NP * RG) for a in (A_k_cache, A_v_cache)]
    vmem = pltpu.VMEM
    out = pl.pallas_call(
        _kernel,
        out_shape=jax.ShapeDtypeStruct((ND, 1, 128), bf16),
        in_specs=[pl.BlockSpec(memory_space=pl.ANY)] * 10,
        out_specs=pl.BlockSpec(memory_space=pltpu.VMEM),
        scratch_shapes=[
            vmem((1, 1, D), bf16), vmem((D,), bf16), vmem((D,), bf16),
            vmem((BUF_ROWS, SEG, 8, 128), bf16),
            vmem((3, 8, 128), f32), vmem((W // 1024, 16, 128), f32),
            vmem((NP * RG, 8, 128), f32), vmem((8, F), f32),
            pltpu.SemaphoreType.DMA((SEM["wo"] + WO_GROUPS,)),
            pltpu.SemaphoreType.DMA((2, N - FINE)),
        ],
        compiler_params=pltpu.CompilerParams(
            vmem_limit_bytes=64 * 1024 * 1024,
            disable_semaphore_checks=True,
        ),
        name="gated_mix_decode",
    )(A_x, gate_w, B_w_r, *caches, _tile_order(A_wq, BIG_LINES), _tile_order(A_wo, BIG_LINES),
      *[_tile_order(a, FFN_SEGS) for a in (B_w_gate, B_w_up, B_w_down)])
    return out.reshape(1, 1, D)
```

```python
import jax
import jax.numpy as jnp
import jax.experimental.pallas as pl
import jax.experimental.pallas.tpu as pltpu

H, DH, SK, D, F = 32, 192, 32768, 640, 1536
W = min(4096, max(256, SK // 4))

SEG = 4
LINE = 64
NP = H // 2
RG = 2 * DH // 8
WSEG = W // 128 // SEG
ND, NQ, NF = D // 128, H * DH // 128, F // 128
BIG_LINES = D * H * DH // (1024 * SEG * LINE)
FFN_SEGS = D * F // (1024 * SEG)
FFN_SHARE = FFN_SEGS // NP
FFN_WAYS = dict(wg=NF // SEG, wu=NF // SEG, wd=ND)

KV_RUN, KV_SWEEP = 6, 12
KV_COLS = ((7, 4), (6, 5), (3, 0), (2, 1))
BIG_RUN = 5
TAIL, TAIL_RUN = 20, 4
SKEW = 26
LAG = 20
END_LAG = 14

f32 = jnp.float32
bf16 = jnp.bfloat16


def _sweep(top, bottom, cols, run):
    return [(r, c, min(run, bottom - r), True) for c in cols for r in range(top, bottom, run)]


def _slots(name, hp, units, riders=()):
    out = []
    for i, (r, c, n, down) in enumerate(units):
        if i < len(riders):
            out.append(((name, hp, r, c, n, down), riders[i]))
        else:
            m = n - 1
            out.append(((name, hp, r, c, m, down), (name, hp, r + m * down, c + m * (not down), n - m, down)))
    return out


def _build_stream():
    kv = [u for cols in KV_COLS for top in range(0, RG, KV_SWEEP)
          for u in _sweep(top, top + KV_SWEEP, cols, KV_RUN)]
    stream, end = [], {}

    def put(name, hp, units):
        ffn = [(w, hp, k, 0, 1, True) for k in range(FFN_SHARE) for w in FFN_WAYS]
        riders = dict(k=ffn[:len(ffn) // 2], v=ffn[len(ffn) // 2:]).get(name, ())
        stream.extend(_slots(name, hp, units, riders))
        end[name, hp] = len(stream)

    put("wq", None, _sweep(0, BIG_LINES, range(LINE), BIG_RUN))
    put("k", 0, kv)
    for hp in range(1, NP):
        put("k", hp, kv)
        put("v", hp - 1, kv)
    put("v", NP - 1, kv)
    put("wo", None, _sweep(0, BIG_LINES, range(LINE - TAIL), BIG_RUN)
        + _sweep(0, BIG_LINES - 1, range(LINE - TAIL, LINE), BIG_RUN)
        + [(BIG_LINES - 1, c, TAIL_RUN, False) for c in range(LINE - TAIL, LINE, TAIL_RUN)])
    return stream, end, len(kv)


STREAM, END, KV_SLOTS = _build_stream()
N = len(STREAM)
WO_START = END["v", NP - 1]
COL_SLOTS = BIG_LINES // BIG_RUN
WO_GROUPS = (LINE - TAIL) // ND
FINE = WO_START + WO_GROUPS * ND * COL_SLOTS

KV_ROWS = RG * WSEG
ROW0 = dict(k=0, v=2 * KV_ROWS, wq=4 * KV_ROWS, wo=4 * KV_ROWS + BIG_LINES * LINE)
ROW0["wg"] = ROW0["wo"] + BIG_LINES * LINE
ROW0["wu"] = ROW0["wg"] + FFN_SEGS
ROW0["wd"] = ROW0["wu"] + FFN_SEGS
BUF_ROWS = ROW0["wd"] + FFN_SEGS
WO_ROW = [ROW0["wo"]]
for _slot in STREAM[WO_START:]:
    WO_ROW.append(WO_ROW[-1] + _slot[0][4] + _slot[1][4])
SEM = dict(k=0, v=2, wq=4, ffn=5, small=6, wo=9)


def _kernel(x_hbm, gw_hbm, wr_hbm, k_hbm, v_hbm, wq, wo, wg, wu, wd, out_ref,
            x_v, gw_v, wr_v, buf, q_s, p_s, o_s, h_s, sems, end_sems):
    src = dict(k=k_hbm, v=v_hbm, wq=wq, wo=wo, wg=wg, wu=wu, wd=wd)

    def kv_row(name, hp):
        return ROW0[name] + (hp & 1) * KV_ROWS

    def wo_row(i, queue):
        return WO_ROW[i - WO_START] + (0 if queue else STREAM[i][0][4])

    def copy(i, queue, step):
        name, hp, r, c, n, down = STREAM[i][1 - queue]
        if name in FFN_WAYS:
            ways = FFN_WAYS[name]
            dst = ROW0[name] + r % ways * (FFN_SEGS // ways) + r // ways + (hp + step) * (FFN_SHARE // ways)
            r, sem = r + (hp + step) * FFN_SHARE, sems.at[SEM["ffn"]]
        elif name == "wq":
            c = c + step
            dst, sem = ROW0[name] + r + c * BIG_LINES, sems.at[SEM[name]]
        elif name == "wo":
            dst = wo_row(i, queue)
            group = (i - WO_START) // (ND * COL_SLOTS)
            sem = end_sems.at[queue, i - FINE] if i >= FINE else sems.at[SEM[name] + group]
        else:
            hp = hp + step
            dst, sem = kv_row(name, hp) + (c * RG + r), sems.at[SEM[name] + (hp & 1)]
            r, c = r + hp * RG, c + LINE - WSEG
        piece = src[name].at[pl.ds(r, n), c] if down else src[name].at[r, pl.ds(c, n)]
        return pltpu.make_async_copy(piece, buf.at[pl.ds(dst, n)], sem)

    def wait_rows(row0, n, sem):
        rows = buf.at[pl.ds(row0, n)]
        pltpu.make_async_copy(rows, rows, sems.at[sem]).wait()

    small = [pltpu.make_async_copy(a, b, sems.at[SEM["small"] + i])
             for i, (a, b) in enumerate(((x_hbm, x_v), (gw_hbm, gw_v), (wr_hbm, wr_v)))]

    row = jax.lax.broadcasted_iota(jnp.int32, (16, 128), 0)
    lane = jax.lax.broadcasted_iota(jnp.int32, (16, 128), 1)
    st = {}

    def accumulate(key, val):
        st[key] = jax.lax.add(st[key], val) if key in st else val

    def matmul(lhs, rhs, contract=0):
        return jax.lax.dot_general(lhs.astype(bf16), rhs, (((1,), (contract,)), ((), ())),
                                   preferred_element_type=f32)

    def kv_matmul(name, hp, g, col, lhs, contract):
        blk = buf[pl.ds(kv_row(name, hp) + (col * RG + g * 16), 16)]
        out = [matmul(jnp.where((row & 7) == (col * SEG + b) % 8, lhs, 0.0), blk[:, b].reshape(128, 128), contract)
               for b in range(SEG)]
        return (out[0] + out[1]) + (out[2] + out[3])

    def every(stride, first, *index):
        rows = buf[(pl.ds(first, (ND - 1) * stride + 1), *index)]
        return jnp.concatenate([jax.lax.index_in_dim(rows, u * stride) for u in range(ND)])

    def own(g):
        return (row < 8, (row < 8) == (lane < DH - 128), row >= 8)[g]

    def t_token(_):
        for c in small:
            c.wait()
        x = x_v[0].astype(f32)
        st["gate"] = jax.nn.sigmoid(jnp.sum(x * gw_v[...].astype(f32).reshape(1, D), axis=-1, keepdims=True))
        st["route"] = jax.nn.sigmoid(jnp.sum(x * wr_v[...].astype(f32).reshape(1, D), axis=-1, keepdims=True))
        st["x"] = jnp.broadcast_to(x, (8, D))

    def t_q(hp, g):
        def fn(step):
            c = 3 * (hp + step) + g
            seg, b = c >> 2, c & (SEG - 1)
            parts = []
            for v in range(16):
                at = seg + v * NQ // SEG
                first = ROW0["wq"] + (at & (LINE - 1)) * BIG_LINES + (at >> 6)
                parts.append(every(BIG_LINES // ND, first, b))
            q_s[g] = matmul(st["x"], jnp.stack(parts, axis=1).reshape(D, 128))
        return fn

    def t_qk(hp, col, g):
        def fn(step):
            q = q_s[g]
            q = jnp.where(own(g), jnp.concatenate([q, q]), 0.0)
            accumulate(("s", col * SEG // 8), kv_matmul("k", hp + step, g, col, q, 0))
        return fn

    def t_softmax(_):
        def per_head(vals, op, reduce):
            v = vals[0]
            for u in vals[1:]:
                v = op(v, u)
            v = reduce(v, axis=1, keepdims=True)
            return jnp.where(row < 8, reduce(v[:8], axis=0, keepdims=True), reduce(v[8:], axis=0, keepdims=True))

        s = [st.pop(("s", cg)) * DH ** -0.5 for cg in range(W // 1024)]
        m = per_head(s, jnp.maximum, jnp.max)
        e = [jnp.exp(v - m) for v in s]
        total = per_head(e, jnp.add, jnp.sum)
        for cg, v in enumerate(e):
            p_s[cg] = v / total

    def t_pv(hp, g, col):
        def fn(step):
            accumulate("o", kv_matmul("v", hp + step, g, col, st["p"][col * SEG // 8], 1))
            if col == WSEG - 1:
                o = jnp.where(own(g), st.pop("o"), 0.0)
                o = jnp.sum(o[:8] + o[8:], axis=0, keepdims=True) * st["gate"]
                o = jnp.broadcast_to(o, (128, 128)).T
                o_s[pl.ds((hp + step) * RG + g * 16, 16)] = o.reshape(16, 8, 128)
                if g == 2:
                    del st["p"]
        return fn

    def t_up(name, c):
        def fn(_):
            w = buf[pl.ds(ROW0[name] + c // SEG * (D // 8), D // 8), c % SEG]
            st[name] = matmul(st["x"], w.reshape(D, 128))
            if name == "wu":
                h_s[:, c * 128:(c + 1) * 128] = jax.nn.silu(st.pop("wg")) * st.pop("wu")
        return fn

    def t_down(j, k):
        def fn(_):
            at = [divmod(ND * v + j, SEG) for v in range(SEG)]
            w = [buf[pl.ds(ROW0["wd"] + way * (FFN_SEGS // ND) + k * 16, 16), b] for way, b in at]
            accumulate("y", matmul(h_s[:, k * 512:(k + 1) * 512], jnp.stack(w, axis=1).reshape(512, 128)))
            if k == F // 512 - 1:
                x = st["x"][:, j * 128:(j + 1) * 128]
                b = x + (x * 0.0 + st.pop("y") * st["route"])
                accumulate(("out", j), jnp.where(row[:8] == 0, (1.0 - st["gate"]) * b, 0.0))
        return fn

    def apply_wo(w, line, col):
        n = w.shape[0] * SEG
        rg, j0 = divmod((line * LINE + col) * SEG, ND)
        groups = pl.cdiv(j0 + n, ND)
        o = jnp.broadcast_to(o_s[pl.ds(rg, groups)][:, None], (groups, ND, 8, 128))
        terms = w.astype(f32).reshape(n, 8, 128) * o.reshape(groups * ND, 8, 128)[j0:j0 + n]
        if n % ND == 0:
            terms = jnp.sum(terms.reshape(n // ND, ND, 8, 128), axis=0)
        for t in range(terms.shape[0]):
            accumulate(("out", (j0 + t) % ND), jax.lax.index_in_dim(terms, t, keepdims=False))

    def t_wo_line(group, line):
        first = ROW0["wo"] + group * ND * BIG_LINES + line
        return lambda _: apply_wo(every(BIG_LINES, first), line, group * ND)

    def wo_piece(i, queue):
        _, _, r, c, n, down = STREAM[i][1 - queue]
        w = buf[pl.ds(wo_row(i, queue), n)]
        if down:
            for k in range(n):
                apply_wo(w[k:k + 1], r + k, c)
        else:
            apply_wo(w, r, c)

    n_slots = N + SKEW + END_LAG
    plan = [[] for _ in range(n_slots)]

    def spread(lo, hi, tasks):
        for k, fn in enumerate(tasks):
            plan[lo + k * (hi - lo) // len(tasks)].append(fn)

    def landed(name, hp):
        return END[name, hp] + SKEW + LAG

    def wait_kv(name, hp):
        return lambda step: wait_rows(kv_row(name, hp + step), KV_ROWS, SEM[name] + ((hp + step) & 1))

    def q_tasks(hp):
        return [t_q(hp, g) for g in range(3)] if hp < NP else []

    def qk_tasks(hp):
        return [wait_kv("k", hp)] + [t_qk(hp, col, g) for col in range(WSEG) for g in range(3)]

    def pv_tasks(hp, first):
        return ([wait_kv("v", hp), lambda _: st.update(p=[p_s[cg] for cg in range(W // 1024)]), first]
                + [t_pv(hp, g, col) for g in range(3) for col in range(WSEG)])

    span = KV_SLOTS - 1
    spread(landed("wq", None), landed("wq", None) + span,
           [lambda _: wait_rows(ROW0["wq"], BIG_LINES * LINE, SEM["wq"]), t_token] + q_tasks(0))
    spread(landed("k", 0), landed("k", 0) + span, qk_tasks(0) + [t_softmax] + q_tasks(1))
    for hp in range(1, NP):
        spread(landed("k", hp), landed("k", hp) + span, qk_tasks(hp))
        spread(landed("v", hp - 1), landed("v", hp - 1) + span, pv_tasks(hp - 1, t_softmax) + q_tasks(hp + 1))
    assert SKEW + LAG + span <= 2 * KV_SLOTS

    mid = landed("v", NP - 1) + 80
    spread(landed("v", NP - 1), mid,
           pv_tasks(NP - 1, lambda _: wait_rows(ROW0["wg"], 3 * FFN_SEGS, SEM["ffn"]))
           + [t_up(w, c) for c in range(NF) for w in ("wg", "wu")]
           + [t_down(j, k) for j in range(ND) for k in range(F // 512)])
    for group in range(WO_GROUPS):
        lo = max(WO_START + (group + 1) * ND * COL_SLOTS + SKEW + LAG, mid + 12 * group)
        plan[lo].append(lambda _, group=group: wait_rows(
            ROW0["wo"] + group * ND * BIG_LINES, ND * BIG_LINES, SEM["wo"] + group))
        spread(lo, lo + 12, [t_wo_line(group, line) for line in range(BIG_LINES)])
    assert mid <= FINE + SKEW + END_LAG <= N

    def run(lo, hi, step=0):
        for i in range(lo, hi):
            done = i - SKEW - END_LAG
            if i < N:
                copy(i, 1, step).start(priority=1)
            if done >= FINE:
                copy(done, 1, step).wait()
            if i == 0 or SKEW < i < N + SKEW:
                copy(max(i - SKEW, 0), 0, step).start(priority=0)
            if i == END["wq", None]:
                for c in small:
                    c.start()
            if done >= FINE:
                copy(done, 0, step).wait()
                wo_piece(done, 0)
                wo_piece(done, 1)
            for fn in plan[i]:
                fn(step)

    def loop(lo, period, count):
        def body(step, carry):
            run(lo, lo + period, step)
            return carry
        jax.lax.fori_loop(0, count, body, 0)
        return lo + period * count

    run(0, SKEW + 1)
    at = loop(SKEW + 1, COL_SLOTS, (END["wq", None] - SKEW - 1) // COL_SLOTS)
    run(at, landed("k", 1))
    at = loop(landed("k", 1), 2 * KV_SLOTS, NP - 2)
    run(at, n_slots)
    for j in range(ND):
        out_ref[j] = jnp.sum(st["out", j], axis=0, keepdims=True).astype(bf16)


def _tile_order(a, lines):
    r, c = a.shape
    return a.reshape(r // 8, 8, c // 128, 128).transpose(0, 2, 1, 3).reshape(lines, -1, SEG, 8, 128)


@jax.jit
def pallas_gated_mix__sliding_block_cached__moe_arch_mod__decode_kernel(
        A_x, A_k_cache, A_v_cache, A_wq, A_wo, B_x, B_w_r, B_w_gate, B_w_up, B_w_down, gate_w):
    del B_x
    caches = [_tile_order(jnp.swapaxes(a, 2, 3).reshape(H * DH, SK), NP * RG) for a in (A_k_cache, A_v_cache)]
    vmem = pltpu.VMEM
    out = pl.pallas_call(
        _kernel,
        out_shape=jax.ShapeDtypeStruct((ND, 1, 128), bf16),
        in_specs=[pl.BlockSpec(memory_space=pl.ANY)] * 10,
        out_specs=pl.BlockSpec(memory_space=pltpu.VMEM),
        scratch_shapes=[
            vmem((1, 1, D), bf16), vmem((D,), bf16), vmem((D,), bf16),
            vmem((BUF_ROWS, SEG, 8, 128), bf16),
            vmem((3, 8, 128), f32), vmem((W // 1024, 16, 128), f32),
            vmem((NP * RG, 8, 128), f32), vmem((8, F), f32),
            pltpu.SemaphoreType.DMA((SEM["wo"] + WO_GROUPS,)),
            pltpu.SemaphoreType.DMA((2, N - FINE)),
        ],
        compiler_params=pltpu.CompilerParams(
            vmem_limit_bytes=64 * 1024 * 1024,
            disable_semaphore_checks=True,
        ),
        name="gated_mix_decode",
    )(A_x, gate_w, B_w_r, *caches, _tile_order(A_wq, BIG_LINES), _tile_order(A_wo, BIG_LINES),
      *[_tile_order(a, FFN_SEGS) for a in (B_w_gate, B_w_up, B_w_down)])
    return out.reshape(1, 1, D)
```
